```python
import jax
import jax.numpy as jnp

def _softmax(x, axis=-1):
    return jax.nn.softmax(x, axis=axis)

def _gelu(x):
    return jax.nn.gelu(x, approximate=True)

def _silu(x):
    return jax.nn.silu(x)

def _sigmoid(x):
    return jax.nn.sigmoid(x)

def _layernorm(x, axis=-1, eps=1e-05):
    m = jnp.mean(x, axis=axis, keepdims=True)
    v = jnp.var(x, axis=axis, keepdims=True)
    return (x - m) / jnp.sqrt(v + eps)

def _scatter_add(tgt, idx, src, axis=0):
    return tgt.at[idx].add(src)

def _segment_sum(src, seg, n):
    return jax.ops.segment_sum(src, seg, n)

class _Rng:

    def __init__(self, key):
        self._k = key

    def _next(self):
        self._k, sub = jax.random.split(self._k)
        return sub

    def normal(self, shape):
        return jax.random.normal(self._next(), shape, dtype=jnp.bfloat16)

    def randint(self, lo, hi, shape):
        return jax.random.randint(self._next(), shape, lo, hi, dtype=jnp.int32)

    def uniform(self, shape, lo=0.0, hi=1.0):
        return jax.random.uniform(self._next(), shape, jnp.bfloat16, lo, hi)

    def permutation(self, n):
        return jax.random.permutation(self._next(), n)
kernel_name = 'sequential_preLN__memory_aug_infini_attn__moe_arch_mod__prompt'

def setup_inputs():
    _rng = _Rng(jax.random.key(int.from_bytes(__import__("os").urandom(4), "little")))
    _w = lambda a: (lambda t: t.astype(jnp.bfloat16) if jnp.issubdtype(t.dtype, jnp.floating) else t)(jnp.asarray(a))

    def _A_setup():
        B, S, D, H = (1, 2048, 576, 32)
        N = 4
        L = max(1, S // N)
        sc = D ** (-0.5)
        return {'x': _w((lambda *s: _rng.normal(s) * 0.05)(B, N * L, D)), 'wq': _w((lambda *s: _rng.normal(s) * 0.05)(D, D) * sc), 'wk': _w((lambda *s: _rng.normal(s) * 0.05)(D, D) * sc), 'wv': _w((lambda *s: _rng.normal(s) * 0.05)(D, D) * sc), 'wo': _w((lambda *s: _rng.normal(s) * 0.05)(D, D) * sc), 'beta': _w((lambda *s: _rng.normal(s) * 0.05)(H))}
    _A_in = _A_setup()

    def _B_setup():
        B, S, D, F, C = (1, 2048, 576, 4608, 1)
        return {'x': _w((lambda *s: _rng.normal(s) * 0.05)(B, S, D)), 'w_r': _w((lambda *s: _rng.normal(s) * 0.05)(D)), 'w_gate': _w((lambda *s: _rng.normal(s) * 0.05)(D, F)), 'w_up': _w((lambda *s: _rng.normal(s) * 0.05)(D, F)), 'w_down': _w((lambda *s: _rng.normal(s) * 0.05)(F, D))}
    _B_in = _B_setup()
    return {'A_x': _A_in['x'], 'A_wq': _A_in['wq'], 'A_wk': _A_in['wk'], 'A_wv': _A_in['wv'], 'A_wo': _A_in['wo'], 'A_beta': _A_in['beta'], 'B_x': _B_in['x'], 'B_w_r': _B_in['w_r'], 'B_w_gate': _B_in['w_gate'], 'B_w_up': _B_in['w_up'], 'B_w_down': _B_in['w_down']}

def reference(A_x, A_wq, A_wk, A_wv, A_wo, A_beta, B_x, B_w_r, B_w_gate, B_w_up, B_w_down):

    def _A_ref(x, wq, wk, wv, wo, beta):
        B, S, D = x.shape
        H = 32
        Dh = D // H
        N = 4
        L = S // N
        q = (lambda x, *d: x.transpose(*d))((x @ wq).reshape(B, S, H, Dh), 0, 2, 1, 3).reshape(B, H, N, L, Dh)
        k = (lambda x, *d: x.transpose(*d))((x @ wk).reshape(B, S, H, Dh), 0, 2, 1, 3).reshape(B, H, N, L, Dh)
        v = (lambda x, *d: x.transpose(*d))((x @ wv).reshape(B, S, H, Dh), 0, 2, 1, 3).reshape(B, H, N, L, Dh)
        phi = lambda t: jnp.where(t > 0, t + 1.0, jnp.exp(t))
        scale = Dh ** (-0.5)
        ar = jnp.arange(L)
        mask = (lambda x, dt: x.astype(dt))(ar[:, None] < ar[None, :], x.dtype) * -1000000000.0
        g = _sigmoid(beta).reshape(1, H, 1, 1)
        M = jnp.einsum('bhd,bhe->bhde', q[:, :, 0, 0, :] * 0.0, q[:, :, 0, 0, :] * 0.0)
        z = q[:, :, 0, 0, :] * 0.0
        outs = []
        for s in range(N):
            qs, ks, vs = (q[:, :, s].copy(), k[:, :, s].copy(), v[:, :, s].copy())
            logits = jnp.einsum('bhqd,bhkd->bhqk', qs, ks) * scale + mask
            p = _softmax(logits, axis=-1)
            a_dot = jnp.einsum('bhqk,bhkd->bhqd', p, vs)
            pq = phi(qs)
            num = jnp.einsum('bhld,bhde->bhle', pq, M)
            den = jnp.einsum('bhld,bhd->bhl', pq, z)[..., None] + 1e-06
            a_mem = num / den
            o = g * a_mem + (1.0 - g) * a_dot
            outs.append(o)
            pk = phi(ks)
            M = M + jnp.einsum('bhld,bhle->bhde', pk, vs)
            z = z + jnp.einsum('bhld->bhd', pk)
        o = (lambda x, *d: x.transpose(*d))(jnp.stack(outs, 2).reshape(B, H, S, Dh), 0, 2, 1, 3).reshape(B, S, D)
        return o @ wo

    def _B_ref(x, w_r, w_gate, w_up, w_down):
        B, S, D = x.shape
        C = 1
        r = x @ w_r
        idx = jnp.argsort(-r, axis=-1)[:, :C]
        idx_e = jnp.repeat(idx.reshape(B, C, 1), D, axis=2)
        x_sel = jnp.take_along_axis(x, idx_e, axis=1)
        g = _silu(x_sel @ w_gate)
        u = x_sel @ w_up
        y = g * u @ w_down
        r_sel = _sigmoid(jnp.take_along_axis(r, idx, axis=1))
        y = y * r_sel.reshape(B, C, 1)
        b_off = (jnp.arange(B) * S).reshape(B, 1)
        flat_idx = (idx + b_off).reshape(B * C)
        zero = (x * 0.0).reshape(B * S, D)
        upd = _scatter_add(zero, flat_idx, y.reshape(B * C, D), axis=0)
        return x + upd.reshape(B, S, D)
    x = A_x
    h = x + _A_ref(_layernorm(x, axis=-1), A_wq, A_wk, A_wv, A_wo, A_beta)
    h2 = h + _B_ref(_layernorm(h, axis=-1), B_w_r, B_w_gate, B_w_up, B_w_down)
    return h2
```

```python
import functools

import jax
import jax.numpy as jnp
from jax import lax
import jax.experimental.pallas as pl
import jax.experimental.pallas.tpu as pltpu

S, D, H, DH, NSEG, L, F = 2048, 576, 32, 18, 4, 512, 4608
HPT = 7
NT = 5
EPS = 1e-5
NEG = -1e30
QSCALE = float(DH ** -0.5 * 1.4426950408889634)

U32, BF16, F32 = jnp.uint32, jnp.bfloat16, jnp.float32


def _b(u):
    return pltpu.bitcast(u, BF16)


def _u(b):
    return pltpu.bitcast(b, U32)


def _phi(t):
    return jnp.where(t > 0, t + 1.0, jnp.exp(t))


def _colsum(a):
    return jnp.sum(a, axis=0, keepdims=True)


def _kernel(x_hbm, wq_hbm, wk_hbm, wv_hbm, wo_hbm, beta_ref, wr_ref, wg_hbm, wu_hbm, wd_hbm,
            out_hbm,
            xs, wraw, wt, wall, wot, xn, qt, pq, kk, pk, vt, ot, den, sbuf, mbuf, bias, gtab, wrc,
            hn, outb, rbuf, wg, wu, wd, sems):
    xu = x_hbm.bitcast(U32)
    ou = out_hbm.bitcast(U32)

    xcp = [pltpu.make_async_copy(xu.at[:, pl.ds(L * s, L)], xs.at[s], sems.at[s]) for s in range(NSEG)]
    wcp = [pltpu.make_async_copy(w.bitcast(U32), wraw.at[i], sems.at[4 + i])
           for i, w in enumerate((wk_hbm, wq_hbm, wv_hbm, wo_hbm))]
    fcp = [pltpu.make_async_copy(w.bitcast(U32), d, sems.at[8 + i])
           for i, (w, d) in enumerate(((wg_hbm, wg), (wu_hbm, wu), (wd_hbm, wd)))]
    xcp[0].start()
    wcp[0].start()
    wcp[1].start()
    wcp[2].start()
    for s in range(1, NSEG):
        xcp[s].start()
    wcp[3].start()
    for c in fcp:
        c.start()

    g_row = jax.nn.sigmoid(beta_ref[...].astype(F32)).reshape(1, H)
    gmat = jnp.broadcast_to(g_row, (128, H)).T
    for h in range(H):
        gtab[h] = gmat[h:h + 1, :]
    wr_row = wr_ref[...].astype(F32).reshape(1, D)
    wrc[...] = jnp.broadcast_to(wr_row, (128, D)).T
    ri = lax.broadcasted_iota(jnp.int32, (128, 128), 0)
    ci = lax.broadcasted_iota(jnp.int32, (128, 128), 1)
    bias[...] = jnp.where(ci >= ri, 0.0, NEG).astype(F32)
    den[0] = jnp.zeros((H, 1, L), F32)
    ot[0] = jnp.zeros((D, L), F32)

    def ln1(s):
        xcp[s].wait()
        for c in range(4):
            xf = _b(xs[s, :, 128 * c:128 * c + 128]).astype(F32)
            mean = _colsum(xf) * (1.0 / D)
            xc = xf - mean
            var = _colsum(xc * xc) * (1.0 / D)
            xn[s, :, 128 * c:128 * c + 128] = _u((xc * lax.rsqrt(var + EPS)).astype(BF16))

    ln1(0)

    def prep_g(i, dst0):
        wcp[i].wait()
        wt[...] = _u(_b(wraw[i]).T)
        for t in range(NT):
            if t < 4:
                v = wt[63 * t:63 * t + 64, :]
                r = lax.broadcasted_iota(jnp.int32, v.shape, 0)
                wall[dst0 + 64 * t:dst0 + 64 * t + 64, :] = jnp.where(r < 63, v, jnp.uint32(0))
            else:
                v = wt[248:288, :]
                r = lax.broadcasted_iota(jnp.int32, v.shape, 0)
                v = wt[252:288, :]
                wall[dst0 + 256:dst0 + 296, :] = jnp.concatenate([v, jnp.zeros((4, D), U32)], axis=0)
                wall[dst0 + 296:dst0 + 320, :] = jnp.zeros((24, D), U32)

    prep_g(0, 0)
    prep_g(1, 320)
    wcp[2].wait()
    wall[640:928, :] = _u(_b(wraw[2]).T)

    for s in range(1, NSEG):
        ln1(s)

    wcp[3].wait()
    wot[...] = _u(_b(wraw[3]).T)

    def proj(s, carry):
        rhs = _b(xn[s])
        kT = jnp.dot(_b(wall[0:320, :]), rhs, preferred_element_type=F32).astype(BF16)
        for t in range(NT):
            kt = kT[128 * t:128 * t + 128, :].T
            kk[s, t] = _u(kt)
            pk[s, t] = _u(_phi(kt.astype(F32)).astype(BF16))
        qT = jnp.dot(_b(wall[320:640, :]), rhs, preferred_element_type=F32)
        for t in range(NT):
            q = qT[128 * t:128 * t + 128, :]
            qt[s, t] = _u((q * QSCALE).astype(BF16))
            pq[s, t] = _u(_phi(q).astype(BF16))
        vT = jnp.dot(_b(wall[640:928, :]), rhs, preferred_element_type=F32)
        vt[s] = _u(vT.astype(BF16))
        return carry

    lax.fori_loop(0, NSEG, proj, 0)

    W0 = [0, 112, 240, 368, 496]
    for t in range(NT):
        w0 = W0[t]
        nw = 144 if t < 4 else 80
        nh = HPT if t < 4 else 4
        rr = lax.broadcasted_iota(jnp.int32, (nw, 128), 0) + w0
        cc = lax.broadcasted_iota(jnp.int32, (nw, 128), 1)
        bd = (rr // DH == HPT * t + cc // DH) & (cc < DH * nh)
        zr = lax.broadcasted_iota(jnp.int32, (16, 128), 0)
        zc = lax.broadcasted_iota(jnp.int32, (16, 128), 1)
        zm = (zr == zc // DH) & (zc < DH * nh)
        C = None
        z = None
        for s in range(NSEG - 1):
            pks = _b(pk[s, t])
            d = jnp.dot(_b(vt[s, w0 // 2:(w0 + nw) // 2, :]), pks, preferred_element_type=F32)
            zs = _colsum(pks.astype(F32))
            C = d if C is None else C + d
            z = zs if z is None else z + zs
            lhs = jnp.concatenate([jnp.where(bd, C, 0.0), jnp.where(zm, jnp.broadcast_to(z, (16, 128)), 0.0)],
                                  axis=0).astype(BF16)
            R = jnp.dot(lhs, _b(pq[s + 1, t]), preferred_element_type=F32)
            for i in range(nh):
                den[s + 1, HPT * t + i] = R[nw + i:nw + i + 1, :]
            ov = 0 if t == 0 else (W0[t - 1] + 144 - w0)
            if ov:
                ot[s + 1, w0:w0 + ov, :] = ot[s + 1, w0:w0 + ov, :] + R[0:ov, :]
            ot[s + 1, w0 + ov:w0 + nw, :] = R[ov:nw, :]

    js = [3, 2, 1, 0]
    steps = [(j, t) for j in js for t in range(j + 1)]
    LAG = 6
    lane = lax.broadcasted_iota(jnp.int32, (8, 128), 1)
    r32 = lax.broadcasted_iota(jnp.int32, (32, 128), 0)
    r16 = lax.broadcasted_iota(jnp.int32, (16, 128), 0)

    def hparams(hp):
        w08 = pl.multiple_of(((hp * DH) // 16) * 8, 8)
        w0 = pl.multiple_of(((hp * DH) // 16) * 16, 16)
        return hp, w0, w08, hp * DH - w0

    def stage(h, do_qk, do_prev, do_cur):
        if do_qk:
            tq = h // HPT
            oq = (h - HPT * tq) * DH
            kmask = jnp.where((lane >= oq) & (lane < oq + DH), jnp.uint32(0xFFFFFFFF), jnp.uint32(0))
        if do_cur:
            pcur = hparams(h)
        if do_prev:
            pprev = hparams(h - 1)
        m8 = [None] * NSEG
        acc = [None] * NSEG

        def qk(q, s):
            j, t = steps[q]
            qm = _b(qt[s, tq, :, 128 * j:128 * j + 128])
            ku = kk[s, tq, 64 * t:64 * t + 64, :]
            ku = (ku.reshape(8, 8, 128) & kmask[None]).reshape(64, 128)
            sc = jnp.dot(_b(ku), qm, preferred_element_type=F32)
            if t == j:
                sc = sc + bias[...]
            sbuf[s, q] = sc
            mx = jnp.max(sc.reshape(16, 8, 128), axis=0)
            m8[s] = mx if t == 0 else jnp.maximum(m8[s], mx)
            if t == j:
                mm = m8[s]
                mm = jnp.maximum(mm, pltpu.roll(mm, 4, 0))
                mm = jnp.maximum(mm, pltpu.roll(mm, 2, 0))
                mm = jnp.maximum(mm, pltpu.roll(mm, 1, 0))
                mbuf[s, j] = mm

        def pv(q, s):
            p = (q - LAG) % 10
            hp, w0, w08, off = pcur if q - LAG >= 0 else pprev
            j, t = steps[p]
            mm = mbuf[s, j]
            sc = sbuf[s, p]
            pr = jnp.exp2(sc.reshape(16, 8, 128) - mm[None]).reshape(128, 128)
            vu = vt[s, pl.ds(w08, 16), 128 * t:128 * t + 128]
            first = off == 0
            rstar = jnp.where(first, 15, 0)
            ones_u = jnp.where(first, jnp.uint32(0x3F800000), jnp.uint32(0x00003F80))
            keep_u = jnp.where(first, jnp.uint32(0x0000FFFF), jnp.uint32(0xFFFF0000))
            vu = jnp.where(r16 == rstar, (vu & keep_u) | ones_u, vu)
            o = jnp.dot(_b(vu), pr.astype(BF16), preferred_element_type=F32)
            acc[s] = o if t == 0 else acc[s] + o
            if t == j:
                a = acc[s]
                l = jnp.where(first, a[31:32, :], a[0:1, :])
                cs = pl.ds(128 * j, 128)
                old = ot[s, pl.ds(w0, 32), cs]
                dn = den[s, hp, :, cs]
                gv = gtab[hp]
                new = a * ((1.0 - gv) / l) + old * (gv / (dn + 1e-6))
                rmask = (r32 >= off) & (r32 < off + DH)
                ot[s, pl.ds(w0, 32), cs] = jnp.where(rmask, new, old)

        for q in range(10):
            for s in range(NSEG):
                if do_qk:
                    qk(q, s)
                if (q - LAG >= 0 and do_cur) or (q - LAG < 0 and do_prev):
                    pv(q, s)

    stage(0, True, False, True)

    def hbody(h, c):
        stage(h, True, True, True)
        return c

    lax.fori_loop(1, H, hbody, 0)
    stage(H, False, True, False)

    ocp = [pltpu.make_async_copy(outb.at[s], ou.at[:, pl.ds(L * s, L)], sems.at[12 + s]) for s in range(NSEG)]

    def post(s, carry):
        attn = jnp.dot(_b(wot[...]), ot[s].astype(BF16), preferred_element_type=F32)
        for c in range(4):
            cs = slice(128 * c, 128 * c + 128)
            hh = _b(xs[s, :, cs]).astype(F32) + attn[:, cs]
            mean = _colsum(hh) * (1.0 / D)
            hc = hh - mean
            var = _colsum(hc * hc) * (1.0 / D)
            hnf = hc * lax.rsqrt(var + EPS)
            hnb = hnf.astype(BF16)
            outb[s, :, cs] = _u((hh + hnf).astype(BF16))
            hn[4 * s + c] = _u(hnb)
            rbuf[s, c:c + 1, :] = _colsum(hnb.astype(F32) * wrc[...])
        pltpu.make_async_copy(outb.at[s], ou.at[:, pl.ds(pl.multiple_of(L * s, L), L)], sems.at[12 + s]).start()
        return carry

    lax.fori_loop(0, NSEG, post, 0)

    R = rbuf[...].reshape(NSEG * 8, 128)
    rr = lax.broadcasted_iota(jnp.int32, R.shape, 0)
    cc = lax.broadcasted_iota(jnp.int32, R.shape, 1)
    valid = (rr % 8) < 4
    R = jnp.where(valid, R, -jnp.inf)
    rmax = jnp.max(R)
    tok = (rr // 8) * L + (rr % 8) * 128 + cc
    idx = jnp.min(jnp.where(valid & (R == rmax), tok, S))
    idx = jnp.minimum(idx, S - 1)
    cb = idx // 128
    ln = idx - cb * 128
    onehot = (lax.broadcasted_iota(jnp.int32, (16, 128), 1) == ln)
    oh = jnp.where(onehot, 1.0, 0.0).astype(BF16)
    xrow = lax.dot_general(oh, _b(hn[cb]), (((1,), (1,)), ((), ())), preferred_element_type=F32).astype(BF16)
    for c in fcp:
        c.wait()
    gate = jnp.dot(xrow, _b(wg[...]), preferred_element_type=F32)
    up = jnp.dot(xrow, _b(wu[...]), preferred_element_type=F32)
    act = (gate * jax.nn.sigmoid(gate) * up).astype(BF16)
    y = lax.dot_general(act, _b(wd[...]), (((1,), (1,)), ((), ())), preferred_element_type=F32)
    y = y * (jax.nn.sigmoid(jnp.full((16, D), rmax, F32)) * (1.0 / 16))
    ycol = lax.dot_general(y.astype(BF16), oh, (((0,), (0,)), ((), ())), preferred_element_type=F32)
    sb = cb // 4
    cl = pl.multiple_of((cb - 4 * sb) * 128, 128)
    for c in ocp:
        c.wait()
    blk = _b(outb[sb, :, pl.ds(cl, 128)]).astype(F32) + ycol
    outb[sb, :, pl.ds(cl, 128)] = _u(blk.astype(BF16))
    fin = pltpu.make_async_copy(outb.at[sb, :, pl.ds(cl, 128)],
                                ou.at[:, pl.ds(pl.multiple_of(cb * 128, 128), 128)], sems.at[16])
    fin.start()
    fin.wait()


@jax.jit
def pallas_sequential_preLN__memory_aug_infini_attn__moe_arch_mod__prompt_kernel(
    A_x: jax.Array,
    A_wq: jax.Array,
    A_wk: jax.Array,
    A_wv: jax.Array,
    A_wo: jax.Array,
    A_beta: jax.Array,
    B_x: jax.Array,
    B_w_r: jax.Array,
    B_w_gate: jax.Array,
    B_w_up: jax.Array,
    B_w_down: jax.Array,
):
    del B_x
    xT = A_x.reshape(S, D).T
    wdT = B_w_down.T
    any_spec = pl.BlockSpec(memory_space=pl.ANY)
    vmem_spec = pl.BlockSpec(memory_space=pltpu.VMEM)
    scratch = [
        pltpu.VMEM((NSEG, D // 2, L), U32),
        pltpu.VMEM((4, D // 2, D), U32),
        pltpu.VMEM((D // 2, D), U32),
        pltpu.VMEM((928, D), U32),
        pltpu.VMEM((D // 2, D), U32),
        pltpu.VMEM((NSEG, D // 2, L), U32),
        pltpu.VMEM((NSEG, NT, 64, L), U32),
        pltpu.VMEM((NSEG, NT, 64, L), U32),
        pltpu.VMEM((NSEG, NT, L // 2, 128), U32),
        pltpu.VMEM((NSEG, NT, L // 2, 128), U32),
        pltpu.VMEM((NSEG, D // 2, L), U32),
        pltpu.VMEM((NSEG, D, L), F32),
        pltpu.VMEM((NSEG, H, 1, L), F32),
        pltpu.VMEM((NSEG, 10, 128, 128), F32),
        pltpu.VMEM((NSEG, 4, 8, 128), F32),
        pltpu.VMEM((128, 128), F32),
        pltpu.VMEM((H, 1, 128), F32),
        pltpu.VMEM((D, 128), F32),
        pltpu.VMEM((16, D // 2, 128), U32),
        pltpu.VMEM((NSEG, D // 2, L), U32),
        pltpu.VMEM((NSEG, 8, 128), F32),
        pltpu.VMEM((D // 2, F), U32),
        pltpu.VMEM((D // 2, F), U32),
        pltpu.VMEM((D // 2, F), U32),
        pltpu.SemaphoreType.DMA((17,)),
    ]
    outT = pl.pallas_call(
        _kernel,
        out_shape=jax.ShapeDtypeStruct((D, S), BF16),
        in_specs=[any_spec] * 5 + [vmem_spec, vmem_spec] + [any_spec] * 3,
        out_specs=any_spec,
        scratch_shapes=scratch,
        compiler_params=pltpu.CompilerParams(vmem_limit_bytes=110 * 1024 * 1024),
    )(xT, A_wq, A_wk, A_wv, A_wo, A_beta, B_w_r, B_w_gate, B_w_up, wdT)
    return outT.T.reshape(1, S, D)
```

```python
import jax
import jax.numpy as jnp
from jax import lax
import jax.experimental.pallas as pl
import jax.experimental.pallas.tpu as pltpu

S, D, H, DH, NSEG, L, F = 2048, 576, 32, 18, 4, 512, 4608
HPT = 7
NT = 5
EPS = 1e-5
NEG = -1e30
QSCALE = float(DH ** -0.5 * 1.4426950408889634)

UNR = 6
FC = 512
MC = 144
NB = 1

U32, BF16, F32 = jnp.uint32, jnp.bfloat16, jnp.float32


def _b(u):
    return pltpu.bitcast(u, BF16)


def _u(b):
    return pltpu.bitcast(b, U32)


def _phi(t):
    return jnp.where(t > 0, t + 1.0, jnp.exp(t))


def _vsum(a, par=4):
    n = a.shape[0] // 8
    par = min(par, n)
    parts = []
    for c in range(par):
        acc = None
        for i in range(c, n, par):
            v = a[8 * i:8 * i + 8]
            acc = v if acc is None else acc + v
        parts.append(acc)
    while len(parts) > 1:
        parts = [parts[i] + parts[i + 1] if i + 1 < len(parts) else parts[i] for i in range(0, len(parts), 2)]
    return parts[0]


def _colsum(a):
    return jnp.sum(_vsum(a), axis=0, keepdims=True)


def _kernel(x_hbm, wq_hbm, wk_hbm, wv_hbm, wo_hbm, beta_ref, wr_ref, wg_hbm, wu_hbm, wd_hbm,
            out_hbm,
            xs, wraw, wt, wall, wot, cw, qt, pq, kk, pk, vt, ot, den, sbuf, mbuf, bias, gtab, wrc,
            hn, outb, wg, wu, wd, yacc, hb0, hb1, st, piv, sems):
    xu = x_hbm.bitcast(U32)
    ou = out_hbm.bitcast(U32)

    def xcp(s):
        return pltpu.make_async_copy(xu.at[:, pl.ds(L * s if isinstance(s, int) else pl.multiple_of(L * s, L), L)], xs.at[s], sems.at[s])

    wcp = [pltpu.make_async_copy(w.bitcast(U32), wraw.at[i], sems.at[4 + i])
           for i, w in enumerate((wk_hbm, wq_hbm, wv_hbm, wo_hbm))]
    fcp = [pltpu.make_async_copy(w.bitcast(U32), d, sems.at[8 + i])
           for i, (w, d) in enumerate(((wg_hbm, wg), (wu_hbm, wu), (wd_hbm, wd)))]
    wcp[0].start()
    xcp(0).start()
    wcp[1].start()
    wcp[2].start()
    wcp[3].start()
    for s in range(1, NSEG):
        xcp(s).start()

    g_row = jax.nn.sigmoid(beta_ref[...].astype(F32)).reshape(1, H)
    gmat = jnp.broadcast_to(g_row, (128, H)).T
    for h in range(H):
        gtab[h] = gmat[h:h + 1, :]
    wr_row = wr_ref[...].astype(F32).reshape(1, D)
    wrc[...] = jnp.broadcast_to(wr_row, (128, D)).T
    ri = lax.broadcasted_iota(jnp.int32, (128, 128), 0)
    ci = lax.broadcasted_iota(jnp.int32, (128, 128), 1)
    bias[...] = jnp.where(ci >= ri, 0.0, NEG).astype(F32)
    for b in range(4):
        den[b] = jnp.zeros((H, 1, 128), F32)
        ot[b] = jnp.zeros((D, 128), F32)

    def zero_of(v):
        return ((v if v.dtype == U32 else pltpu.bitcast(v, U32)) >> 31) >> 1

    def stats(s):
        rs, ms = [], []
        for c in range(4):
            xf = _b(xs[s, :, 128 * c:128 * c + 128]).astype(F32)
            p = xf[0:1, :]
            d = xf - p
            m1 = _colsum(d) * (1.0 / D)
            var = _colsum(d * d) * (1.0 / D) - m1 * m1
            mean = p + m1
            r = lax.rsqrt(jnp.maximum(var, 0.0) + EPS)
            piv[:, pl.ds(128 * c if isinstance(s, int) else pl.multiple_of(L * s + 128 * c, 128), 128)] = jnp.broadcast_to(mean, (8, 128))
            rs.append(jnp.broadcast_to(r, (8, 128)))
            ms.append(jnp.broadcast_to(mean * r, (8, 128)))
        return jnp.concatenate(rs, axis=1), jnp.concatenate(ms, axis=1)

    def prep_g(i, dst0):
        wcp[i].wait()
        wt[...] = _u(_b(wraw[i]).T)
        for t in range(NT):
            if t < 4:
                v = wt[63 * t:63 * t + 64, :]
                r = lax.broadcasted_iota(jnp.int32, v.shape, 0)
                wall[dst0 + 64 * t:dst0 + 64 * t + 64, :] = jnp.where(r < 63, v, jnp.uint32(0))
            else:
                v = wt[252:288, :]
                wall[dst0 + 256:dst0 + 296, :] = jnp.concatenate([v, jnp.zeros((4, D), U32)], axis=0)

    def rowsum(lo, hi):
        w = _b(wall[lo:hi, :]).astype(F32)
        cw[2 * lo:2 * hi, :] = jnp.broadcast_to(jnp.sum(w, axis=1, keepdims=True), (2 * (hi - lo), 128))

    prep_g(0, 0)
    rowsum(0, 296)

    def prep_q():
        prep_g(1, 296)
        rowsum(296, 592)

    def prep_v():
        wcp[2].wait()
        wcp[3].wait()
        wall[592:880, :] = _u(_b(wraw[2]).T)
        wot[...] = _u(_b(wraw[3]).T)
        rowsum(592, 880)

    for c in fcp:
        c.start()
    for s in range(NSEG):
        qt[296:320, L * s:L * s + L] = jnp.zeros((24, L), U32)
        pq[296:320, L * s:L * s + L] = jnp.zeros((24, L), U32)

    def proj(s, carry, first=False):
        xcp(s).wait()
        scs = pl.ds(0 if first else pl.multiple_of(L * s, L), L)
        srs = pl.ds(0 if first else pl.multiple_of(256 * s, 256), 256)
        rhs = _b(xs[s])
        rstd, mr = stats(s)

        def lnmm(lo, hi):
            a = jnp.dot(_b(wall[lo:hi, :]), rhs, preferred_element_type=F32)
            n = 2 * (hi - lo)
            c = cw[2 * lo:2 * hi, :].reshape(n // 8, 8, 128)
            c = jnp.concatenate([c] * 4, axis=2)
            return (a.reshape(n // 8, 8, L) * rstd[None] - c * mr[None]).reshape(n, L)

        kT = lnmm(0, 296).astype(BF16)
        for t in range(NT):
            if t < 4:
                kt = kT[128 * t:128 * t + 128, :].T
            else:
                kt = jnp.concatenate([kT[512:592, :], jnp.zeros((48, L), BF16)], axis=0).T
            kk[srs, 128 * t:128 * t + 128] = _u(kt)
            pk[srs, 128 * t:128 * t + 128] = _u(_phi(kt.astype(F32)).astype(BF16))
        if first:
            prep_q()
        qT = lnmm(296, 592)
        for t in range(NT):
            n = 128 if t < 4 else 80
            q = qT[128 * t:128 * t + n, :]
            qt[64 * t:64 * t + n // 2, scs] = _u((q * QSCALE).astype(BF16))
            pq[64 * t:64 * t + n // 2, scs] = _u(_phi(q).astype(BF16))
        if first:
            prep_v()
        vT = lnmm(592, 880)
        vt[s] = vT.astype(BF16).astype(F32)
        return carry

    proj(0, 0, True)
    lax.fori_loop(1, NSEG, proj, 0)


    W0 = [0, 120, 248, 376, 504]
    WN = [128, 136, 136, 128, 72]
    for t in range(NT):
        w0, nw = W0[t], WN[t]
        nh = HPT if t < 4 else 4
        rr = lax.broadcasted_iota(jnp.int32, (nw, 128), 0) + w0
        cc = lax.broadcasted_iota(jnp.int32, (nw, 128), 1)
        bd = (rr // DH == HPT * t + cc // DH) & (cc < DH * nh)
        zr = lax.broadcasted_iota(jnp.int32, (8, 128), 0)
        zc = lax.broadcasted_iota(jnp.int32, (8, 128), 1)
        zm = (zr == zc // DH) & (zc < DH * nh)
        C = None
        z = None
        for s in range(NSEG - 1):
            pks = _b(pk[256 * s:256 * s + 256, 128 * t:128 * t + 128])
            d = jnp.dot(vt[s, w0:w0 + nw, :], pks, preferred_element_type=F32)
            zs = _colsum(pks.astype(F32))
            C = d if C is None else C + d
            z = zs if z is None else z + zs
            lhs = jnp.concatenate([jnp.where(bd, C, 0.0), jnp.where(zm, jnp.broadcast_to(z, (8, 128)), 0.0)], axis=0)
            R = jnp.dot(lhs, _b(pq[64 * t:64 * t + 64, L * (s + 1):L * (s + 2)]), preferred_element_type=F32)
            ov = 0 if t == 0 else (W0[t - 1] + WN[t - 1] - w0)
            for c in range(4):
                b = 4 * (s + 1) + c
                cs = slice(128 * c, 128 * c + 128)
                for i in range(nh):
                    den[b, HPT * t + i] = R[nw + i:nw + i + 1, cs]
                if ov:
                    ot[b, w0:w0 + ov, :] = ot[b, w0:w0 + ov, :] + R[0:ov, cs]
                ot[b, w0 + ov:w0 + nw, :] = R[ov:nw, cs]

    js = [3, 2, 1, 0]
    steps = [(j, t) for j in js for t in range(j + 1)]
    LAG = 6
    lane = lax.broadcasted_iota(jnp.int32, (8, 128), 1)
    r24 = lax.broadcasted_iota(jnp.int32, (24, 128), 0)
    r8 = lax.broadcasted_iota(jnp.int32, (8, 128), 0)

    def hparams(hp):
        w0 = ((hp * DH) >> 3) << 3
        if not isinstance(hp, int):
            w0 = pl.multiple_of(w0, 8)
        return hp, w0, hp * DH - w0

    def stage(h, do_qk, do_prev, do_cur):
        if do_qk:
            tq = (h * 37) >> 8
            oq = (h - HPT * tq) * DH
            if isinstance(h, int):
                qrs, kcs = pl.ds(64 * tq, 64), pl.ds(128 * tq, 128)
            else:
                qrs = pl.ds(pl.multiple_of(64 * tq, 64), 64)
                kcs = pl.ds(pl.multiple_of(128 * tq, 128), 128)
            kmask = jnp.where((lane >= oq) & (lane < oq + DH), jnp.uint32(0xFFFFFFFF), jnp.uint32(0))
        if do_cur:
            pcur = hparams(h)
        if do_prev:
            pprev = hparams(h - 1)
        m8 = [None] * NSEG
        acc = [None] * NSEG

        def qk(q, s):
            j, t = steps[q]
            qm = _b(qt[qrs, L * s + 128 * j:L * s + 128 * j + 128])
            ku = kk[256 * s + 64 * t:256 * s + 64 * t + 64, kcs]
            ku = (ku.reshape(8, 8, 128) & kmask[None]).reshape(64, 128)
            sc = jnp.dot(_b(ku), qm, preferred_element_type=F32)
            if t == j:
                sc = sc + bias[...]
            sbuf[s, q] = sc
            mx = jnp.max(sc.reshape(16, 8, 128), axis=0)
            m8[s] = mx if t == 0 else jnp.maximum(m8[s], mx)
            if t == j:
                mm = m8[s]
                mm = jnp.maximum(mm, pltpu.roll(mm, 4, 0))
                mm = jnp.maximum(mm, pltpu.roll(mm, 2, 0))
                mm = jnp.maximum(mm, pltpu.roll(mm, 1, 0))
                mbuf[s, j] = mm

        def pv(q, s):
            p = (q - LAG) % 10
            hp, w0, off = pcur if q - LAG >= 0 else pprev
            j, t = steps[p]
            mm = mbuf[s, j]
            sc = sbuf[s, p]
            pr = jnp.exp2(sc.reshape(16, 8, 128) - mm[None]).reshape(128, 128)
            v = vt[s, pl.ds(w0, 24), 128 * t:128 * t + 128]
            first = off == 0
            v = jnp.concatenate([
                jnp.where((r8 == 0) & jnp.logical_not(first), 1.0, v[0:8]),
                v[8:16],
                jnp.where((r8 == 7) & first, 1.0, v[16:24])], axis=0)
            o = jnp.dot(v, pr.astype(BF16), preferred_element_type=F32)
            acc[s] = o if t == 0 else acc[s] + o
            if t == j:
                a = acc[s]
                l = jnp.where(first, a[23:24, :], a[0:1, :])
                b = 4 * s + j
                old = ot[b, pl.ds(w0, 24), :]
                dn = den[b, hp]
                gv = gtab[hp]
                new = (a * ((1.0 - gv) * pl.reciprocal(l, approx=True))
                       + old * (gv * pl.reciprocal(dn + 1e-6, approx=True)))
                rmask = (r24 >= off) & (r24 < off + DH)
                ot[b, pl.ds(w0, 24), :] = jnp.where(rmask, new, old)

        for q in range(10):
            for s in range(NSEG):
                if do_qk:
                    qk(q, s)
                if (q - LAG >= 0 and do_cur) or (q - LAG < 0 and do_prev):
                    pv(q, s)

    stage(0, True, False, True)
    npeel = (H - 1) % UNR
    for h in range(1, 1 + npeel):
        stage(h, True, True, True)

    def hbody(i, c):
        for u in range(UNR):
            stage(1 + npeel + UNR * i + u, True, True, True)
        return c

    lax.fori_loop(0, (H - 1) // UNR, hbody, 0)
    stage(H, False, True, False)

    NM = D // MC

    def post_step(go, gl, best, par):
        hbo, hbl = (hb0, hb1) if par == 0 else (hb1, hb0)
        NW = 128 * NB
        if go is not None:
            s = (go * NB) >> 2
            cs = pl.ds(pl.multiple_of(((go * NB) & 3) * 128, NW), NW)
            gcs = pl.ds(pl.multiple_of(go * NW, NW), NW)
            ob = jnp.concatenate([ot[go * NB + u] for u in range(NB)], axis=1).astype(BF16)
            c0 = piv[:, gcs]
            hcs_o = pl.ds(pl.multiple_of((go >> 1) * NW, NW), NW)
            s1 = s2 = None
        if gl is not None:
            bcs = pl.ds(pl.multiple_of(gl * NW, NW), NW)
            hcs_l = pl.ds(pl.multiple_of((gl >> 1) * NW, NW), NW)
            m1 = jnp.sum(st[0:8, bcs], axis=0, keepdims=True) * (1.0 / D)
            var = jnp.sum(st[8:16, bcs], axis=0, keepdims=True) * (1.0 / D) - m1 * m1
            mean = jnp.broadcast_to(piv[0:1, bcs] + m1, (8, NW))
            rstd = jnp.broadcast_to(lax.rsqrt(jnp.maximum(var, 0.0) + EPS), (8, NW))
            r = None
        for m in range(NM):
            rows = slice(MC * m, MC * (m + 1))
            urows = slice(MC // 2 * m, MC // 2 * (m + 1))
            if go is not None:
                a = jnp.dot(_b(wot[urows, :]), ob, preferred_element_type=F32)
                hm = a + _b(xs[s, urows, cs]).astype(F32)
                hbo[rows, hcs_o] = hm
                d = (hm.reshape(MC // 8, 8, NW) - c0[None]).reshape(MC, NW)
                t1, t2 = _vsum(d, 2), _vsum(d * d, 2)
                s1 = t1 if s1 is None else s1 + t1
                s2 = t2 if s2 is None else s2 + t2
            if gl is not None:
                hh = hbl[rows, hcs_l]
                hnf = ((hh.reshape(MC // 8, 8, NW) - mean[None]) * rstd[None]).reshape(MC, NW)
                outb[urows, bcs] = _u((hh + hnf).astype(BF16))
                hn[urows, bcs] = _u(hnf.astype(BF16))
                w = wrc[rows, :]
                t = _vsum(hnf * jnp.concatenate([w] * NB, axis=1), 2)
                r = t if r is None else r + t
                if go is not None and m + 1 < NM:
                    ob = jnp.concatenate([_b(_u(ob[0:16]) | zero_of(t)), ob[16:]], axis=0)
        if go is not None:
            st[0:8, gcs] = s1
            st[8:16, gcs] = s2
        if gl is not None:
            r = jnp.sum(r, axis=0, keepdims=True)
            bv, bi = best
            for u in range(NB):
                ru = r[:, 128 * u:128 * u + 128]
                upd = ru > bv
                bv, bi = jnp.where(upd, ru, bv), jnp.where(upd, gl * NB + u, bi)
            best = (bv, bi)
        return best

    def ocp(s):
        return pltpu.make_async_copy(outb.at[:, pl.ds(pl.multiple_of(L * s, L), L)], ou.at[:, pl.ds(pl.multiple_of(L * s, L), L)], sems.at[12 + s])

    best = (jnp.full((1, 128), -jnp.inf, F32), jnp.zeros((1, 128), jnp.int32))
    NG = 16 // NB
    best = post_step(0, None, best, 0)

    def post(i, best):
        best = post_step(2 * i + 1, 2 * i, best, 1)
        best = post_step(2 * i + 2, 2 * i + 1, best, 0)
        bl = (2 * i + 1) * NB + NB - 1

        @pl.when((bl & 3) == 3)
        def _():
            ocp(bl >> 2).start()

        return best

    best = lax.fori_loop(0, NG // 2 - 1, post, best)
    best = post_step(NG - 1, NG - 2, best, 1)
    best = post_step(None, NG - 1, best, 0)
    ocp(3).start()

    bv, bi = best
    c128 = lax.broadcasted_iota(jnp.int32, (1, 128), 1)
    rmax = jnp.max(bv)
    idx = jnp.min(jnp.where(bv == rmax, bi * 128 + c128, S))
    idx = jnp.minimum(idx, S - 1)
    cb = idx >> 7
    ln = idx & 127
    ccs = pl.ds(pl.multiple_of(cb * 128, 128), 128)
    onehot = (lax.broadcasted_iota(jnp.int32, (16, 128), 1) == ln)
    oh = jnp.where(onehot, 1.0, 0.0).astype(BF16)
    xrow = lax.dot_general(oh, _b(hn[:, ccs]), (((1,), (1,)), ((), ())), preferred_element_type=F32)[0:8]
    for c in fcp:
        c.wait()
    NG = F // FC

    def gate_up(c):
        cs = pl.ds(FC * c, FC)
        gate = jnp.dot(xrow, _b(wg[:, cs]), preferred_element_type=F32)
        up = jnp.dot(xrow, _b(wu[:, cs]), preferred_element_type=F32)
        act = gate * jax.nn.sigmoid(gate) * up
        return act.astype(BF16).astype(F32)

    def down(c, act):
        for f in range(D // 16):
            a0 = a1 = None
            for k in range(FC // 128):
                w = _b(wd[8 * f:8 * f + 8, FC * c + 128 * k:FC * c + 128 * k + 128]).astype(F32)
                ak = act[:, 128 * k:128 * k + 128]
                p0 = w[0:8] * ak
                p1 = w[8:16] * ak
                a0 = p0 if a0 is None else a0 + p0
                a1 = p1 if a1 is None else a1 + p1
            a = jnp.concatenate([a0, a1], axis=0)
            if c == 0:
                yacc[16 * f:16 * f + 16, :] = a
            else:
                yacc[16 * f:16 * f + 16, :] = yacc[16 * f:16 * f + 16, :] + a

    act = gate_up(0)
    for c in range(NG):
        nxt = gate_up(c + 1) if c + 1 < NG else None
        down(c, act)
        act = nxt
    ycol = jnp.sum(yacc[...], axis=1, keepdims=True)
    ycol = ycol.astype(BF16).astype(F32) * jax.nn.sigmoid(jnp.full((D, 128), rmax, F32))
    ycol = jnp.where(lax.broadcasted_iota(jnp.int32, (D, 128), 1) == ln, ycol, 0.0)
    for s in range(NSEG):
        ocp(s).wait()
    blk = _b(outb[:, ccs]).astype(F32) + ycol
    outb[:, ccs] = _u(blk.astype(BF16))
    fin = pltpu.make_async_copy(outb.at[:, ccs], ou.at[:, ccs], sems.at[16])
    fin.start()
    fin.wait()


@jax.jit
def pallas_sequential_preLN__memory_aug_infini_attn__moe_arch_mod__prompt_kernel(
    A_x: jax.Array,
    A_wq: jax.Array,
    A_wk: jax.Array,
    A_wv: jax.Array,
    A_wo: jax.Array,
    A_beta: jax.Array,
    B_x: jax.Array,
    B_w_r: jax.Array,
    B_w_gate: jax.Array,
    B_w_up: jax.Array,
    B_w_down: jax.Array,
):
    del B_x
    xT = A_x.reshape(S, D).T
    wdT = B_w_down.T
    any_spec = pl.BlockSpec(memory_space=pl.ANY)
    vmem_spec = pl.BlockSpec(memory_space=pltpu.VMEM)
    scratch = [
        pltpu.VMEM((NSEG, D // 2, L), U32),
        pltpu.VMEM((4, D // 2, D), U32),
        pltpu.VMEM((D // 2, D), U32),
        pltpu.VMEM((880, D), U32),
        pltpu.VMEM((D // 2, D), U32),
        pltpu.VMEM((1760, 128), F32),
        pltpu.VMEM((NT * 64, S), U32),
        pltpu.VMEM((NT * 64, S), U32),
        pltpu.VMEM((S // 2, NT * 128), U32),
        pltpu.VMEM((S // 2, NT * 128), U32),
        pltpu.VMEM((NSEG, D, L), F32),
        pltpu.VMEM((16, D, 128), F32),
        pltpu.VMEM((16, H, 1, 128), F32),
        pltpu.VMEM((NSEG, 10, 128, 128), F32),
        pltpu.VMEM((NSEG, 4, 8, 128), F32),
        pltpu.VMEM((128, 128), F32),
        pltpu.VMEM((H, 1, 128), F32),
        pltpu.VMEM((D, 128), F32),
        pltpu.VMEM((D // 2, S), U32),
        pltpu.VMEM((D // 2, S), U32),
        pltpu.VMEM((D // 2, F), U32),
        pltpu.VMEM((D // 2, F), U32),
        pltpu.VMEM((D // 2, F), U32),
        pltpu.VMEM((D, 128), F32),
        pltpu.VMEM((D, S // 2), F32),
        pltpu.VMEM((D, S // 2), F32),
        pltpu.VMEM((16, S), F32),
        pltpu.VMEM((8, S), F32),
        pltpu.SemaphoreType.DMA((17,)),
    ]
    outT = pl.pallas_call(
        _kernel,
        out_shape=jax.ShapeDtypeStruct((D, S), BF16),
        in_specs=[any_spec] * 5 + [vmem_spec, vmem_spec] + [any_spec] * 3,
        out_specs=any_spec,
        scratch_shapes=scratch,
        compiler_params=pltpu.CompilerParams(vmem_limit_bytes=110 * 1024 * 1024),
    )(xT, A_wq, A_wk, A_wv, A_wo, A_beta, B_w_r, B_w_gate, B_w_up, wdT)
    return outT.T.reshape(1, S, D)
```
